```python
import os as _os
_os.environ.setdefault("JAX_PLATFORMS", "cpu")
import jax
import jax.numpy as jnp

def _softmax(x, axis=-1):
    return jax.nn.softmax(x, axis=axis)
def _gelu(x):
    return jax.nn.gelu(x, approximate=True)
def _silu(x):
    return jax.nn.silu(x)
def _sigmoid(x):
    return jax.nn.sigmoid(x)
def _layernorm(x, axis=-1, eps=1e-5):
    m = jnp.mean(x, axis=axis, keepdims=True)
    v = jnp.var(x, axis=axis, keepdims=True)
    return (x - m) / jnp.sqrt(v + eps)
def _scatter_add(tgt, idx, src, axis=0):
    return tgt.at[idx].add(src)
def _segment_sum(src, seg, n):
    return jax.ops.segment_sum(src, seg, n)
class _Rng:
    def __init__(self, key):
        self._k = key
    def _next(self):
        self._k, sub = jax.random.split(self._k)
        return sub
    def normal(self, shape):
        return jax.random.normal(self._next(), shape, dtype=jnp.bfloat16)
    def randint(self, lo, hi, shape):
        return jax.random.randint(self._next(), shape, lo, hi, dtype=jnp.int32)
    def uniform(self, shape, lo=0.0, hi=1.0):
        return jax.random.uniform(self._next(), shape, jnp.bfloat16, lo, hi)
    def permutation(self, n):
        return jax.random.permutation(self._next(), n)


kernel_name = 'standalone__grn__sampling'

def setup_inputs():
    _rng = _Rng(jax.random.key(int.from_bytes(__import__("os").urandom(4), "little")))
    _w = (lambda a: (lambda t: t.astype(jnp.bfloat16) if jnp.issubdtype(t.dtype, jnp.floating) else t)(jnp.asarray(a)))
    B, S, D = 512, 32, 640
    return {
        "x": _w((lambda *s: _rng.normal(s) * 0.05)(B, S, D)),
        "g": _w((lambda *s: _rng.normal(s) * 0.1)(D) * 0.1),
        "b": _w((lambda *s: _rng.normal(s) * 0.1)(D) * 0.1),
    }

def reference(x, g, b):
    gx = jnp.sqrt((x * x).sum(axis=-2, keepdims=True))
    nx = gx / (gx.mean(axis=-1, keepdims=True) + 1e-6)
    return g * (x * nx) + b + x
```

```python
import jax
import jax.numpy as jnp
from jax import lax
import jax.experimental.pallas as pl
import jax.experimental.pallas.tpu as pltpu

_STREAMS = 8
_LOOKAHEAD = 4
_LEAD = 1
_FIRST = 8


@jax.jit
def pallas_standalone__grn__sampling_kernel(
    x: jax.Array,
    g: jax.Array,
    b: jax.Array,
):
    B, S, D = x.shape
    K = _STREAMS
    m = B // K
    shape = (K, m, S, D)

    def kernel(x_hbm, g_hbm, b_hbm, o_hbm, buf, g_v, b_v, rsem, wsem, psem):
        def rd(j):
            return pltpu.make_async_copy(
                x_hbm.at[:, j], buf.at[:, j], rsem.at[lax.rem(j, _LOOKAHEAD)])

        def wr(j):
            return pltpu.make_async_copy(buf.at[:, j], o_hbm.at[:, j], wsem)

        rd(0).start()
        cg = pltpu.make_async_copy(g_hbm, g_v, psem)
        cb = pltpu.make_async_copy(b_hbm, b_v, psem)
        cg.start()
        cb.start()
        for j in range(1, _LOOKAHEAD):
            rd(j).start()
        cg.wait()
        cb.wait()
        gf = jnp.broadcast_to(g_v[...].astype(jnp.float32).reshape(1, D), (8, D))
        bf = jnp.broadcast_to(b_v[...].astype(jnp.float32).reshape(1, D), (8, D))

        def one(k, j):
            xv = buf[k, j].astype(jnp.float32).reshape(S // 8, 8, D)
            ss = jnp.sum(jnp.sum(xv * xv, axis=0), axis=0, keepdims=True)
            gx = jnp.sqrt(ss)
            den = jnp.sum(gx, axis=-1, keepdims=True) * (1.0 / D) + 1e-6
            sc = gf * (gx / den) + 1.0
            buf[k, j] = (xv * sc[None] + bf[None]).reshape(S, D).astype(buf.dtype)

        def body(j, _):
            rd(j).wait()

            @pl.when(j + _LOOKAHEAD < m)
            def _():
                rd(j + _LOOKAHEAD).start()

            @pl.when(j == m - 1 - _LEAD)
            def _():
                lax.fori_loop(0, _FIRST, lambda i, _: wr(i).start(), None)

            for k in range(K):
                one(k, j)

        lax.fori_loop(0, m, body, None)
        lax.fori_loop(_FIRST, m, lambda i, _: wr(i).start(), None)
        pltpu.make_async_copy(buf, o_hbm, wsem).wait()

    out = pl.pallas_call(
        kernel,
        in_specs=[pl.BlockSpec(memory_space=pl.ANY)] * 3,
        out_specs=pl.BlockSpec(memory_space=pl.ANY),
        out_shape=jax.ShapeDtypeStruct(shape, x.dtype),
        scratch_shapes=[
            pltpu.VMEM(shape, x.dtype),
            pltpu.VMEM((D,), g.dtype),
            pltpu.VMEM((D,), b.dtype),
            pltpu.SemaphoreType.DMA((_LOOKAHEAD,)),
            pltpu.SemaphoreType.DMA(()),
            pltpu.SemaphoreType.DMA(()),
        ],
        compiler_params=pltpu.CompilerParams(vmem_limit_bytes=48 * 2**20),
    )(x.reshape(shape), g, b)
    return out.reshape(x.shape)
```

```python
import jax
import jax.numpy as jnp
from jax import lax
import jax.experimental.pallas as pl
import jax.experimental.pallas.tpu as pltpu

_K = 8
_AHEAD = 16
_LEAD = 3
_FIRST = 8
_ROWS = 16


@jax.jit
def pallas_standalone__grn__sampling_kernel(
    x: jax.Array,
    g: jax.Array,
    b: jax.Array,
):
    B, S, D = x.shape
    n = B // _K
    shape = (_K, n, S, D)

    def kernel(x_hbm, g_hbm, b_hbm, o_hbm, buf, g_v, b_v, wsem):
        def start_step(src, dst, j, sem, per):
            for h in range(S // _ROWS):
                for q in range(_K // per):
                    ix = (pl.ds(q * per, per), j, pl.ds(h * _ROWS, _ROWS))
                    pltpu.make_async_copy(src.at[ix], dst.at[ix], sem).start(
                        priority=q % 2)

        def wr(j, _=None):
            start_step(buf, o_hbm, j, wsem, 4)

        def read_and_compute(rsem, psem):
            def rd(j, _=None):
                start_step(x_hbm, buf, j, rsem.at[j & (_AHEAD - 1)], 2)

            def rd_wait(j, _=None):
                pltpu.make_async_copy(
                    x_hbm.at[:, j], buf.at[:, j], rsem.at[j & (_AHEAD - 1)]).wait()

            rd(0)
            cg = pltpu.make_async_copy(g_hbm, g_v, psem)
            cb = pltpu.make_async_copy(b_hbm, b_v, psem)
            cg.start()
            cb.start(priority=1)
            lax.fori_loop(1, _AHEAD, rd, None)
            cg.wait()
            cb.wait()
            gf = jnp.broadcast_to(g_v[...].astype(jnp.float32).reshape(1, D), (_K, D))
            bf = jnp.broadcast_to(b_v[...].astype(jnp.float32).reshape(1, D), (8, D))

            def compute(j):
                row = lax.broadcasted_iota(jnp.int32, (_K, D), 0)
                ss = None
                for k in range(_K):
                    xv = buf[k, j].astype(jnp.float32).reshape(S // 8, 8, D)
                    p = jnp.sum(jnp.sum(xv * xv, axis=0), axis=0, keepdims=True)
                    ss = jnp.broadcast_to(p, (_K, D)) if ss is None else jnp.where(row == k, p, ss)
                gx = jnp.sqrt(ss)
                den = jnp.sum(gx, axis=-1, keepdims=True) * (1.0 / D) + 1e-6
                sc = gf * (gx / den) + 1.0
                for k in range(_K):
                    xv = buf[k, j].astype(jnp.float32).reshape(S // 8, 8, D)
                    s = jnp.broadcast_to(sc[k:k + 1], (8, D))
                    buf[k, j] = (xv * s[None] + bf[None]).reshape(S, D).astype(buf.dtype)

            t = n - _AHEAD

            def body(j, _):
                @pl.when(j < t)
                def _():
                    rd_wait(j)
                    rd(j + _AHEAD)

                @pl.when(j == t)
                def _():
                    lax.fori_loop(t, n - _LEAD, rd_wait, None)
                    lax.fori_loop(0, _FIRST, wr, None)
                    lax.fori_loop(n - _LEAD, n, rd_wait, None)

                @pl.when(j > t)
                def _():
                    wr(_FIRST + j - t - 1)

                compute(j)

            lax.fori_loop(0, n, body, None)
            lax.fori_loop(_FIRST + _AHEAD - 1, n, wr, None)

        pl.run_scoped(
            read_and_compute,
            pltpu.SemaphoreType.DMA((_AHEAD,)),
            pltpu.SemaphoreType.DMA(()),
        )
        pltpu.make_async_copy(buf, o_hbm, wsem).wait()

    out = pl.pallas_call(
        kernel,
        in_specs=[pl.BlockSpec(memory_space=pl.ANY)] * 3,
        out_specs=pl.BlockSpec(memory_space=pl.ANY),
        out_shape=jax.ShapeDtypeStruct(shape, x.dtype),
        scratch_shapes=[
            pltpu.VMEM(shape, x.dtype),
            pltpu.VMEM((D,), g.dtype),
            pltpu.VMEM((D,), b.dtype),
            pltpu.SemaphoreType.DMA(()),
        ],
        compiler_params=pltpu.CompilerParams(vmem_limit_bytes=48 * 2**20),
    )(x.reshape(shape), g, b)
    return out.reshape(x.shape)
```

```python
import jax
import jax.numpy as jnp
from jax import lax
import jax.experimental.pallas as pl
import jax.experimental.pallas.tpu as pltpu

_EPS = 1e-6
_K = 8
_AHEAD = 16
_HEAD = 4
_LEAD = 3
_FIRST = 8
_PER = 2
_RD_ROWS = 16


@jax.jit
def pallas_standalone__grn__sampling_kernel(
    x: jax.Array,
    g: jax.Array,
    b: jax.Array,
):
    B, S, D = x.shape
    assert B % _K == 0 and S % _RD_ROWS == 0
    n = B // _K
    t = n - _AHEAD
    assert t >= _FIRST
    shape = (_K, n, S, D)

    def kernel(x_hbm, g_hbm, b_hbm, o_hbm, buf, g_vmem, b_vmem, wsem):
        def start_step(src, dst, j, sem, rows, priority=None):
            for r in range(0, S, rows):
                for q in range(_K // _PER):
                    ix = (pl.ds(q * _PER, _PER), j, pl.ds(r, rows))
                    pltpu.make_async_copy(src.at[ix], dst.at[ix], sem).start(
                        priority=q % 2 if priority is None else priority)

        def write(j, _=None):
            start_step(buf, o_hbm, j, wsem, S)

        def read_and_normalise(rsem, psem):
            def read(j, _=None, priority=None):
                start_step(x_hbm, buf, j, rsem.at[j & (_AHEAD - 1)], _RD_ROWS,
                           priority)

            def wait_read(j, _=None):
                pltpu.make_async_copy(
                    x_hbm.at[:, j], buf.at[:, j], rsem.at[j & (_AHEAD - 1)]
                ).wait()

            lax.fori_loop(0, _HEAD, lambda j, _: read(j, priority=1), None)
            g_copy = pltpu.make_async_copy(g_hbm, g_vmem, psem)
            b_copy = pltpu.make_async_copy(b_hbm, b_vmem, psem)
            g_copy.start()
            b_copy.start()
            lax.fori_loop(_HEAD, _AHEAD, read, None)
            g_copy.wait()
            b_copy.wait()
            gamma = jnp.broadcast_to(
                g_vmem[...].astype(jnp.float32).reshape(1, D), (_K, D))
            beta = jnp.broadcast_to(
                b_vmem[...].astype(jnp.float32).reshape(1, D), (8, D))

            def load(k, j):
                return buf[k, j].astype(jnp.float32).reshape(S // 8, 8, D)

            def normalise(j):
                row = lax.broadcasted_iota(jnp.int32, (_K, D), 0)
                ssq = jnp.zeros((_K, D), jnp.float32)
                for k in range(_K):
                    xk = load(k, j)
                    part = jnp.sum(
                        jnp.sum(xk * xk, axis=0), axis=0, keepdims=True)
                    ssq = jnp.where(row == k, part, ssq)
                gx = jnp.sqrt(ssq)
                mean = jnp.sum(gx, axis=-1, keepdims=True) * (1.0 / D)
                scale = gamma * (gx / (mean + _EPS)) + 1.0
                for k in range(_K):
                    sk = jnp.broadcast_to(scale[k:k + 1], (8, D))
                    yk = load(k, j) * sk[None] + beta[None]
                    buf[k, j] = yk.reshape(S, D).astype(buf.dtype)

            def step(j, _):
                @pl.when(j < t)
                def _():
                    wait_read(j)
                    read(j + _AHEAD)

                @pl.when(j == t)
                def _():
                    lax.fori_loop(t, n - _LEAD, wait_read, None)
                    lax.fori_loop(0, _FIRST, write, None)
                    lax.fori_loop(n - _LEAD, n, wait_read, None)

                @pl.when(j > t)
                def _():
                    write(_FIRST + j - t - 1)

                normalise(j)

            lax.fori_loop(0, n, step, None)
            lax.fori_loop(_FIRST + _AHEAD - 1, n, write, None)

        pl.run_scoped(
            read_and_normalise,
            pltpu.SemaphoreType.DMA((_AHEAD,)),
            pltpu.SemaphoreType.DMA(()),
        )
        pltpu.make_async_copy(buf, o_hbm, wsem).wait()

    out = pl.pallas_call(
        kernel,
        in_specs=[pl.BlockSpec(memory_space=pl.ANY)] * 3,
        out_specs=pl.BlockSpec(memory_space=pl.ANY),
        out_shape=jax.ShapeDtypeStruct(shape, x.dtype),
        scratch_shapes=[
            pltpu.VMEM(shape, x.dtype),
            pltpu.VMEM((D,), g.dtype),
            pltpu.VMEM((D,), b.dtype),
            pltpu.SemaphoreType.DMA(()),
        ],
        compiler_params=pltpu.CompilerParams(vmem_limit_bytes=48 * 2**20),
    )(x.reshape(shape), g, b)
    return out.reshape(x.shape)
```
